```python
import os as _os
_os.environ.setdefault("JAX_PLATFORMS", "cpu")
import jax
import jax.numpy as jnp

def _softmax(x, axis=-1):
    return jax.nn.softmax(x, axis=axis)
def _gelu(x):
    return jax.nn.gelu(x, approximate=True)
def _silu(x):
    return jax.nn.silu(x)
def _sigmoid(x):
    return jax.nn.sigmoid(x)
def _layernorm(x, axis=-1, eps=1e-5):
    m = jnp.mean(x, axis=axis, keepdims=True)
    v = jnp.var(x, axis=axis, keepdims=True)
    return (x - m) / jnp.sqrt(v + eps)
def _scatter_add(tgt, idx, src, axis=0):
    return tgt.at[idx].add(src)
def _segment_sum(src, seg, n):
    return jax.ops.segment_sum(src, seg, n)
class _Rng:
    def __init__(self, key):
        self._k = key
    def _next(self):
        self._k, sub = jax.random.split(self._k)
        return sub
    def normal(self, shape):
        return jax.random.normal(self._next(), shape, dtype=jnp.bfloat16)
    def randint(self, lo, hi, shape):
        return jax.random.randint(self._next(), shape, lo, hi, dtype=jnp.int32)
    def uniform(self, shape, lo=0.0, hi=1.0):
        return jax.random.uniform(self._next(), shape, jnp.bfloat16, lo, hi)
    def permutation(self, n):
        return jax.random.permutation(self._next(), n)


kernel_name = 'standalone__instancenorm__sampling'

def setup_inputs():
    _rng = _Rng(jax.random.key(int.from_bytes(__import__("os").urandom(4), "little")))
    _w = (lambda a: (lambda t: t.astype(jnp.bfloat16) if jnp.issubdtype(t.dtype, jnp.floating) else t)(jnp.asarray(a)))
    B, C, H, W = 16, 640, 16, 32
    return {
        "x": _w((lambda *s: _rng.normal(s) * 0.05)(B, C, H, W)),
        "g": _w((lambda *s: _rng.normal(s) * 0.05)(C) + 1.0),
        "b": _w((lambda *s: _rng.normal(s) * 0.05)(C)),
    }

def reference(x, g, b):
    mu = x.mean(axis=(-2, -1), keepdims=True)
    var = ((x - mu) * (x - mu)).mean(axis=(-2, -1), keepdims=True)
    xhat = (x - mu) / jnp.sqrt(var + 1e-5)
    return xhat * g.reshape(1, -1, 1, 1) + b.reshape(1, -1, 1, 1)
```

```python
import jax
import jax.numpy as jnp
from jax import lax
import jax.experimental.pallas as pl
import jax.experimental.pallas.tpu as pltpu

_EPS = 1e-5
_HEAD = 14


def _instancenorm_body(x_hbm, g_hbm, b_hbm, o_hbm, xbuf, obuf, gbuf, bbuf, rsem, wsem, psem):
    B, HW, C = xbuf.shape

    def read(i):
        return pltpu.make_async_copy(x_hbm.at[i], xbuf.at[i], rsem.at[i])

    def write(start, n, slot):
        return pltpu.make_async_copy(
            obuf.at[pl.ds(start, n)], o_hbm.at[pl.ds(start, n)], wsem.at[slot])

    copy_g = pltpu.make_async_copy(g_hbm, gbuf, psem.at[0])
    copy_b = pltpu.make_async_copy(b_hbm, bbuf, psem.at[1])
    copy_g.start()
    copy_b.start()

    @pl.loop(0, B)
    def _(i):
        read(i).start()

    copy_g.wait()
    copy_b.wait()
    gv = gbuf[...].astype(jnp.float32).reshape(1, C)
    bv = bbuf[...].astype(jnp.float32).reshape(1, C)

    @pl.loop(0, B)
    def _(i):
        read(i).wait()

        @pl.when(i == _HEAD)
        def _():
            write(0, _HEAD, 0).start()

        xv = xbuf[i].astype(jnp.float32)
        mu = jnp.mean(xv, axis=0, keepdims=True)
        d = xv - mu
        var = jnp.mean(d * d, axis=0, keepdims=True)
        scale = gv * lax.rsqrt(var + _EPS)
        obuf[i] = (d * scale + bv).astype(obuf.dtype)

    write(_HEAD, B - _HEAD, 1).start()
    write(0, _HEAD, 0).wait()
    write(_HEAD, B - _HEAD, 1).wait()


@jax.jit
def pallas_standalone__instancenorm__sampling_kernel(
    x: jax.Array,
    g: jax.Array,
    b: jax.Array,
):
    B, C, H, W = x.shape
    xt = jnp.transpose(x, (0, 2, 3, 1)).reshape(B, H * W, C)

    out = pl.pallas_call(
        _instancenorm_body,
        in_specs=[pl.BlockSpec(memory_space=pl.ANY)] * 3,
        out_specs=pl.BlockSpec(memory_space=pl.ANY),
        out_shape=jax.ShapeDtypeStruct((B, H * W, C), x.dtype),
        scratch_shapes=[
            pltpu.VMEM((B, H * W, C), x.dtype),
            pltpu.VMEM((B, H * W, C), x.dtype),
            pltpu.VMEM((C,), g.dtype),
            pltpu.VMEM((C,), b.dtype),
            pltpu.SemaphoreType.DMA((B,)),
            pltpu.SemaphoreType.DMA((2,)),
            pltpu.SemaphoreType.DMA((2,)),
        ],
        compiler_params=pltpu.CompilerParams(vmem_limit_bytes=64 * 1024 * 1024),
    )(xt, g, b)
    return jnp.transpose(out.reshape(B, H, W, C), (0, 3, 1, 2))
```

```python
import jax
import jax.numpy as jnp
from jax import lax
import jax.experimental.pallas as pl
import jax.experimental.pallas.tpu as pltpu

_EPS = 1e-5
_PIECE = 16
_SPLIT = 128


def _instancenorm_body(x_hbm, g_hbm, b_hbm, o_hbm, xbuf, obuf, gbuf, bbuf, rsem, tsem, wsem):
    J, _, HW, C = xbuf.shape
    n_pieces = HW // _PIECE

    def read(j, h):
        return pltpu.make_async_copy(x_hbm.at[j, h], xbuf.at[j, h], rsem.at[h])

    def read_last(start, size, sem):
        rows = pl.ds(start, size)
        return pltpu.make_async_copy(x_hbm.at[J - 1, 1, rows], xbuf.at[J - 1, 1, rows], sem)

    def write(h, p):
        rows = pl.ds(p * _PIECE, _PIECE)
        return pltpu.make_async_copy(obuf.at[:, h, rows], o_hbm.at[:, h, rows], wsem.at[0])

    def normalize(j, h, gv, bv):
        xv = xbuf[j, h].astype(jnp.float32)
        mu = jnp.mean(xv, axis=0, keepdims=True)
        d = xv - mu
        var = jnp.mean(d * d, axis=0, keepdims=True)
        scale = gv * lax.rsqrt(var + _EPS)
        obuf[j, h] = (d * scale + bv).astype(obuf.dtype)

    copy_g = pltpu.make_async_copy(g_hbm, gbuf, rsem.at[0])
    copy_b = pltpu.make_async_copy(b_hbm, bbuf, rsem.at[0])
    copy_g.start()
    copy_b.start()

    @pl.loop(0, J)
    def _(j):
        read(j, 0).start()

    @pl.loop(0, J - 1)
    def _(j):
        read(j, 1).start()

    read_last(0, _SPLIT, rsem.at[1]).start()
    read_last(_SPLIT, HW - _SPLIT, tsem.at[0]).start()

    copy_g.wait()
    copy_b.wait()

    @pl.loop(0, J)
    def _(j):
        read(j, 0).wait()

    gv = gbuf[...].astype(jnp.float32).reshape(1, C)
    bv = bbuf[...].astype(jnp.float32).reshape(1, C)

    @pl.loop(0, J)
    def _(j):
        normalize(j, 0, gv, bv)

    @pl.loop(0, J - 1)
    def _(j):
        read(j, 1).wait()

    read_last(0, _SPLIT, rsem.at[1]).wait()

    @pl.loop(0, n_pieces)
    def _(p):
        write(0, p).start()

    read_last(_SPLIT, HW - _SPLIT, tsem.at[0]).wait()

    @pl.loop(0, J)
    def _(j):
        normalize(j, 1, gv, bv)

    @pl.loop(0, n_pieces)
    def _(p):
        write(1, p).start()

    for h in range(2):
        @pl.loop(0, n_pieces)
        def _(p):
            write(h, p).wait()


@jax.jit
def pallas_standalone__instancenorm__sampling_kernel(
    x: jax.Array,
    g: jax.Array,
    b: jax.Array,
):
    B, C, H, W = x.shape
    assert B % 2 == 0 and (H * W) % _PIECE == 0 and _SPLIT < H * W
    view = (B // 2, 2, H * W, C)
    xt = jnp.transpose(x, (0, 2, 3, 1)).reshape(view)

    out = pl.pallas_call(
        _instancenorm_body,
        in_specs=[pl.BlockSpec(memory_space=pl.ANY)] * 3,
        out_specs=pl.BlockSpec(memory_space=pl.ANY),
        out_shape=jax.ShapeDtypeStruct(view, x.dtype),
        scratch_shapes=[
            pltpu.VMEM(view, x.dtype),
            pltpu.VMEM(view, x.dtype),
            pltpu.VMEM((C,), g.dtype),
            pltpu.VMEM((C,), b.dtype),
            pltpu.SemaphoreType.DMA((2,)),
            pltpu.SemaphoreType.DMA((1,)),
            pltpu.SemaphoreType.DMA((1,)),
        ],
        compiler_params=pltpu.CompilerParams(vmem_limit_bytes=64 * 1024 * 1024),
    )(xt, g, b)
    return jnp.transpose(out.reshape(B, H, W, C), (0, 3, 1, 2))
```

```python
import jax
import jax.numpy as jnp
from jax import lax
import jax.experimental.pallas as pl
import jax.experimental.pallas.tpu as pltpu

_EPS = 1e-5
_SLAB = 16
_LEAD = 128


def _instancenorm_body(x_hbm, g_hbm, b_hbm, o_hbm, xbuf, obuf, gbuf, bbuf, sems):
    J, _, HW, C = xbuf.shape
    n_slabs = HW // _SLAB
    sem_a, sem_b = sems.at[0], sems.at[1]

    def read(j, h, sem):
        return pltpu.make_async_copy(x_hbm.at[j, h], xbuf.at[j, h], sem)

    def read_last(start, size, sem):
        rows = pl.ds(start, size)
        return pltpu.make_async_copy(x_hbm.at[J - 1, 1, rows], xbuf.at[J - 1, 1, rows], sem)

    def write(h, p):
        rows = pl.ds(p * _SLAB, _SLAB)
        return pltpu.make_async_copy(obuf.at[:, h, rows], o_hbm.at[:, h, rows], sem_b)

    def normalize(j, h, gv, bv):
        xv = xbuf[j, h].astype(jnp.float32)
        mu = jnp.mean(xv, axis=0, keepdims=True)
        d = xv - mu
        var = jnp.mean(d * d, axis=0, keepdims=True)
        scale = gv * lax.rsqrt(var + _EPS)
        obuf[j, h] = (d * scale + bv).astype(obuf.dtype)

    copy_g = pltpu.make_async_copy(g_hbm, gbuf, sem_a)
    copy_b = pltpu.make_async_copy(b_hbm, bbuf, sem_a)
    copy_g.start()
    copy_b.start()

    @pl.loop(0, J)
    def _(j):
        read(j, 0, sem_a).start()

    @pl.loop(0, J - 1)
    def _(j):
        read(j, 1, sem_b).start()

    read_last(0, _LEAD, sem_b).start()

    copy_g.wait()
    copy_b.wait()

    @pl.loop(0, J)
    def _(j):
        read(j, 0, sem_a).wait()

    read_last(_LEAD, HW - _LEAD, sem_a).start()

    gv = gbuf[...].astype(jnp.float32).reshape(1, C)
    bv = bbuf[...].astype(jnp.float32).reshape(1, C)

    @pl.loop(0, J)
    def _(j):
        normalize(j, 0, gv, bv)

    @pl.loop(0, J - 1)
    def _(j):
        read(j, 1, sem_b).wait()

    read_last(0, _LEAD, sem_b).wait()

    @pl.loop(0, n_slabs)
    def _(p):
        write(0, p).start()

    read_last(_LEAD, HW - _LEAD, sem_a).wait()

    @pl.loop(0, J)
    def _(j):
        normalize(j, 1, gv, bv)

    @pl.loop(0, n_slabs)
    def _(p):
        write(1, p).start()

    for h in range(2):
        @pl.loop(0, n_slabs)
        def _(p):
            write(h, p).wait()


@jax.jit
def pallas_standalone__instancenorm__sampling_kernel(
    x: jax.Array,
    g: jax.Array,
    b: jax.Array,
):
    B, C, H, W = x.shape
    assert B % 2 == 0 and (H * W) % _SLAB == 0 and _LEAD % _SLAB == 0 and _LEAD < H * W
    view = (B // 2, 2, H * W, C)
    xt = jnp.transpose(x, (0, 2, 3, 1)).reshape(view)

    out = pl.pallas_call(
        _instancenorm_body,
        in_specs=[pl.BlockSpec(memory_space=pl.ANY)] * 3,
        out_specs=pl.BlockSpec(memory_space=pl.ANY),
        out_shape=jax.ShapeDtypeStruct(view, x.dtype),
        scratch_shapes=[
            pltpu.VMEM(view, x.dtype),
            pltpu.VMEM(view, x.dtype),
            pltpu.VMEM((C,), g.dtype),
            pltpu.VMEM((C,), b.dtype),
            pltpu.SemaphoreType.DMA((2,)),
        ],
        compiler_params=pltpu.CompilerParams(vmem_limit_bytes=64 * 1024 * 1024),
    )(xt, g, b)
    return jnp.transpose(out.reshape(B, H, W, C), (0, 3, 1, 2))
```
